```python
import jax
import jax.numpy as jnp

def _softmax(x, axis=-1):
    return jax.nn.softmax(x, axis=axis)

def _gelu(x):
    return jax.nn.gelu(x, approximate=True)

def _silu(x):
    return jax.nn.silu(x)

def _sigmoid(x):
    return jax.nn.sigmoid(x)

def _layernorm(x, axis=-1, eps=1e-05):
    m = jnp.mean(x, axis=axis, keepdims=True)
    v = jnp.var(x, axis=axis, keepdims=True)
    return (x - m) / jnp.sqrt(v + eps)

def _scatter_add(tgt, idx, src, axis=0):
    return tgt.at[idx].add(src)

def _segment_sum(src, seg, n):
    return jax.ops.segment_sum(src, seg, n)

class _Rng:

    def __init__(self, key):
        self._k = key

    def _next(self):
        self._k, sub = jax.random.split(self._k)
        return sub

    def normal(self, shape):
        return jax.random.normal(self._next(), shape, dtype=jnp.bfloat16)

    def randint(self, lo, hi, shape):
        return jax.random.randint(self._next(), shape, lo, hi, dtype=jnp.int32)

    def uniform(self, shape, lo=0.0, hi=1.0):
        return jax.random.uniform(self._next(), shape, jnp.bfloat16, lo, hi)

    def permutation(self, n):
        return jax.random.permutation(self._next(), n)
kernel_name = 'standalone__dilated_atrous__vision'

def setup_inputs():
    _rng = _Rng(jax.random.key(int.from_bytes(__import__("os").urandom(4), "little")))
    _w = lambda a: (lambda t: t.astype(jnp.bfloat16) if jnp.issubdtype(t.dtype, jnp.floating) else t)(jnp.asarray(a))
    H = W = 384
    C = 384
    k = 1
    return {'x': _w((lambda *s: _rng.normal(s) * 0.05)(1, H, W, C)), 'w': _w((lambda *s: _rng.normal(s) * 0.05)(k, k, C, C) * (1.0 / (k * C ** 0.5)))}

def reference(x, w):
    B, H, W, C = x.shape
    k = 1
    rate = 2
    pad = (k - 1) * rate // 2
    xp = jnp.pad(x, ((0, 0), (pad, pad), (pad, pad), (0, 0)))
    out = jnp.zeros_like(x)
    for i in range(k):
        for j in range(k):
            tap = xp[:, i * rate:i * rate + H, j * rate:j * rate + W, :].copy()
            out = out + jnp.einsum('bhwc,co->bhwo', tap, w[i, j])
    return out
```

```python
import jax
import jax.numpy as jnp
import jax.experimental.pallas as pl
import jax.experimental.pallas.tpu as pltpu


def _mm_kernel(x_ref, w_ref, o_ref):
    o_ref[...] = jnp.dot(
        x_ref[...], w_ref[...], preferred_element_type=jnp.float32
    ).astype(o_ref.dtype)


@jax.jit
def pallas_standalone__dilated_atrous__vision_kernel(x: jax.Array, w: jax.Array):
    B, H, W, C = x.shape
    CO = w.shape[-1]
    M = B * H * W
    bm = 4608
    x2 = x.reshape(M, C)
    w2 = w.reshape(C, CO)
    out = pl.pallas_call(
        _mm_kernel,
        grid=(M // bm,),
        in_specs=[
            pl.BlockSpec((bm, C), lambda i: (i, 0)),
            pl.BlockSpec((C, CO), lambda i: (0, 0)),
        ],
        out_specs=pl.BlockSpec((bm, CO), lambda i: (i, 0)),
        out_shape=jax.ShapeDtypeStruct((M, CO), x.dtype),
        compiler_params=pltpu.CompilerParams(
            dimension_semantics=("parallel",),
            vmem_limit_bytes=100 * 1024 * 1024,
        ),
    )(x2, w2)
    return out.reshape(B, H, W, CO)
```

```python
import jax
import jax.numpy as jnp
import jax.experimental.pallas as pl
import jax.experimental.pallas.tpu as pltpu

_STREAMS = 6
_WRITE_ROWS = 48
_BLOCK_ROWS = 384
_WRITES_AHEAD = 24
_WRITES_PER_STEP = 13


def _conv1x1_kernel(x_hbm, w_hbm, o_hbm, buf, w_vmem, read_sems, w_sem, write_sem):
    streams, length, _ = buf.shape
    n_blocks = length // _BLOCK_ROWS
    n_writes = length // _WRITE_ROWS
    writes_per_block = _BLOCK_ROWS // _WRITE_ROWS
    n_early = (n_blocks * 17) // 32
    n_paced = _WRITES_AHEAD + _WRITES_PER_STEP * (n_blocks - n_early)
    assert n_paced <= n_writes
    assert all(
        _WRITES_AHEAD + _WRITES_PER_STEP * (i - n_early + 1) <= i * writes_per_block
        for i in range(n_early, n_blocks)
    )

    def rows(i, n):
        return pl.ds(pl.multiple_of(i * n, n), n)

    def read(i):
        r = rows(i, _BLOCK_ROWS)
        return pltpu.make_async_copy(x_hbm.at[:, r], buf.at[:, r], read_sems.at[i])

    def write(j):
        r = rows(j, _WRITE_ROWS)
        return pltpu.make_async_copy(buf.at[:, r], o_hbm.at[:, r], write_sem)

    def compute(i):
        r = rows(i, _BLOCK_ROWS)
        for s in range(streams):
            buf[s, r, :] = jnp.dot(
                buf[s, r, :], w_vmem[...], preferred_element_type=jnp.float32
            ).astype(buf.dtype)

    w_copy = pltpu.make_async_copy(w_hbm, w_vmem, w_sem)
    w_copy.start()

    @pl.loop(0, n_blocks)
    def _(i):
        read(i).start()

    w_copy.wait()

    @pl.loop(0, n_early)
    def _(i):
        read(i).wait()
        compute(i)

    @pl.loop(n_early, n_blocks - 1)
    def _(i):
        read(i).wait()

    @pl.loop(0, _WRITES_AHEAD)
    def _(j):
        write(j).start()

    read(n_blocks - 1).wait()

    @pl.loop(n_early, n_blocks)
    def _(i):
        first = _WRITES_AHEAD + (i - n_early) * _WRITES_PER_STEP
        for u in range(_WRITES_PER_STEP):
            write(first + u).start()
        compute(i)

    @pl.loop(n_paced, n_writes)
    def _(j):
        write(j).start()

    pltpu.make_async_copy(buf, o_hbm, write_sem).wait()


@jax.jit
def pallas_standalone__dilated_atrous__vision_kernel(x: jax.Array, w: jax.Array):
    B, H, W, C = x.shape
    assert w.shape == (1, 1, C, C), "1x1 kernel with as many outputs as inputs"
    pixels = B * H * W
    length = pixels // _STREAMS
    assert length * _STREAMS == pixels and length % _BLOCK_ROWS == 0

    out = pl.pallas_call(
        _conv1x1_kernel,
        in_specs=[
            pl.BlockSpec(memory_space=pl.ANY),
            pl.BlockSpec(memory_space=pl.ANY),
        ],
        out_specs=pl.BlockSpec(memory_space=pl.ANY),
        out_shape=jax.ShapeDtypeStruct((_STREAMS, length, C), x.dtype),
        scratch_shapes=[
            pltpu.VMEM((_STREAMS, length, C), x.dtype),
            pltpu.VMEM((C, C), w.dtype),
            pltpu.SemaphoreType.DMA((length // _BLOCK_ROWS,)),
            pltpu.SemaphoreType.DMA,
            pltpu.SemaphoreType.DMA,
        ],
        compiler_params=pltpu.CompilerParams(vmem_limit_bytes=124 * 1024 * 1024),
    )(x.reshape(_STREAMS, length, C), w.reshape(C, C))
    return out.reshape(B, H, W, C)
```

```python
import jax
import jax.numpy as jnp
import jax.experimental.pallas as pl
import jax.experimental.pallas.tpu as pltpu

_STREAMS = 6
_WRITE_ROWS = 48
_BLOCK_ROWS = 384
_TAIL_ROWS = 96
_WRITES_AHEAD = 24
_WRITES_PER_STEP = 13


def _conv1x1_kernel(x_hbm, w_hbm, o_hbm, buf, w_vmem, read_sems, aux_sem):
    streams, length, _ = buf.shape
    n_blocks = length // _BLOCK_ROWS
    n_writes = length // _WRITE_ROWS
    n_first = (n_blocks * 6) // 32
    n_early = (n_blocks * 15) // 32
    bounds = (
        0,
        n_first * _BLOCK_ROWS,
        n_early * _BLOCK_ROWS,
        length - _TAIL_ROWS,
        length,
    )
    assert all(lo < hi for lo, hi in zip(bounds, bounds[1:]))
    n_paced = _WRITES_AHEAD + _WRITES_PER_STEP * (n_blocks - n_early)
    assert n_paced <= n_writes
    assert all(
        (_WRITES_AHEAD + _WRITES_PER_STEP * (i - n_early + 1)) * _WRITE_ROWS
        <= i * _BLOCK_ROWS
        for i in range(n_early, n_blocks)
    )

    def rows(i, n):
        return pl.ds(pl.multiple_of(i * n, n), n)

    def read(k):
        r = pl.ds(bounds[k], bounds[k + 1] - bounds[k])
        return pltpu.make_async_copy(x_hbm.at[:, r], buf.at[:, r], read_sems.at[k % 2])

    def write(j):
        r = rows(j, _WRITE_ROWS)
        return pltpu.make_async_copy(buf.at[:, r], o_hbm.at[:, r], aux_sem)

    def compute(i):
        r = rows(i, _BLOCK_ROWS)
        for s in range(streams):
            buf[s, r, :] = jnp.dot(
                buf[s, r, :], w_vmem[...], preferred_element_type=jnp.float32
            ).astype(buf.dtype)

    w_copy = pltpu.make_async_copy(w_hbm, w_vmem, aux_sem)
    w_copy.start()
    read(0).start()
    read(1).start()
    w_copy.wait()

    read(0).wait()
    read(2).start()
    pl.loop(0, n_first)(compute)

    read(1).wait()
    read(3).start()
    pl.loop(n_first, n_early)(compute)

    read(2).wait()

    @pl.loop(0, _WRITES_AHEAD)
    def _(j):
        write(j).start()

    read(3).wait()

    @pl.loop(n_early, n_blocks)
    def _(i):
        first = _WRITES_AHEAD + (i - n_early) * _WRITES_PER_STEP
        for u in range(_WRITES_PER_STEP):
            write(first + u).start()
        compute(i)

    @pl.loop(n_paced, n_writes)
    def _(j):
        write(j).start()

    pltpu.make_async_copy(buf, o_hbm, aux_sem).wait()


@jax.jit
def pallas_standalone__dilated_atrous__vision_kernel(x: jax.Array, w: jax.Array):
    B, H, W, C = x.shape
    assert w.shape == (1, 1, C, C), "1x1 kernel with as many outputs as inputs"
    pixels = B * H * W
    length = pixels // _STREAMS
    assert length * _STREAMS == pixels
    assert length % _BLOCK_ROWS == 0 and length % _WRITE_ROWS == 0

    out = pl.pallas_call(
        _conv1x1_kernel,
        in_specs=[
            pl.BlockSpec(memory_space=pl.ANY),
            pl.BlockSpec(memory_space=pl.ANY),
        ],
        out_specs=pl.BlockSpec(memory_space=pl.ANY),
        out_shape=jax.ShapeDtypeStruct((_STREAMS, length, C), x.dtype),
        scratch_shapes=[
            pltpu.VMEM((_STREAMS, length, C), x.dtype),
            pltpu.VMEM((C, C), w.dtype),
            pltpu.SemaphoreType.DMA((2,)),
            pltpu.SemaphoreType.DMA,
        ],
        compiler_params=pltpu.CompilerParams(vmem_limit_bytes=118 * 1024 * 1024),
    )(x.reshape(_STREAMS, length, C), w.reshape(C, C))
    return out.reshape(B, H, W, C)
```

```python
import jax
import jax.numpy as jnp
import jax.experimental.pallas as pl
import jax.experimental.pallas.tpu as pltpu

_STREAMS = 6
_BLOCK_ROWS = 384
_READ_ROWS = 32
_GROUP_ROWS = 2 * _BLOCK_ROWS
_GROUPS_AHEAD = 3
_TAIL_ROWS = 192
_WRITE_ROWS = 48
_WRITES_AHEAD = 24
_WRITES_PER_STEP = 13


def _conv1x1_kernel(x_hbm, w_hbm, o_hbm, buf, w_vmem, read_sems, aux_sem):
    streams, length, _ = buf.shape
    half = streams // 2
    n_blocks = length // _BLOCK_ROWS
    n_groups = length // _GROUP_ROWS
    n_writes = length // _WRITE_ROWS
    n_early = n_groups - _GROUPS_AHEAD
    n_paced = _WRITES_AHEAD + _WRITES_PER_STEP * (n_blocks - n_early)
    assert n_early >= 0 and n_paced <= n_writes
    assert _GROUP_ROWS % _READ_ROWS == 0 and _TAIL_ROWS % _READ_ROWS == 0
    assert _BLOCK_ROWS <= _GROUP_ROWS - _TAIL_ROWS
    assert all(
        (_WRITES_AHEAD + _WRITES_PER_STEP * (i - n_early + 1)) * _WRITE_ROWS
        <= i * _BLOCK_ROWS
        for i in range(n_early, n_blocks)
    )

    def rows(start, size, align):
        return pl.ds(pl.multiple_of(start, align), size)

    def group_start(g):
        return g * _GROUP_ROWS - _TAIL_ROWS

    def start_read(g, start):
        r = rows(start, _READ_ROWS, _READ_ROWS)
        for p in range(2):
            s = pl.ds(p * half, half)
            pltpu.make_async_copy(
                x_hbm.at[s, r], buf.at[s, r], read_sems.at[g % _GROUPS_AHEAD]
            ).start(priority=p)

    def start_group(g, start, size):
        @pl.loop(0, size // _READ_ROWS)
        def _(u):
            start_read(g, start + u * _READ_ROWS)

    def wait_group(g, start, size):
        r = rows(start, size, _READ_ROWS)
        pltpu.make_async_copy(
            x_hbm.at[:, r], buf.at[:, r], read_sems.at[g % _GROUPS_AHEAD]
        ).wait()

    def start_write(j):
        r = rows(j * _WRITE_ROWS, _WRITE_ROWS, _WRITE_ROWS)
        pltpu.make_async_copy(buf.at[:, r], o_hbm.at[:, r], aux_sem).start()

    def compute(i):
        r = rows(i * _BLOCK_ROWS, _BLOCK_ROWS, _BLOCK_ROWS)
        for s in range(streams):
            buf[s, r, :] = jnp.dot(
                buf[s, r, :], w_vmem[...], preferred_element_type=jnp.float32
            ).astype(buf.dtype)

    w_copy = pltpu.make_async_copy(w_hbm, w_vmem, aux_sem)
    w_copy.start()
    start_group(0, 0, _GROUP_ROWS - _TAIL_ROWS)
    for g in range(1, _GROUPS_AHEAD):
        start_group(g, group_start(g), _GROUP_ROWS)
    w_copy.wait()
    wait_group(0, 0, _GROUP_ROWS - _TAIL_ROWS)

    @pl.loop(0, n_early)
    def _(i):
        g = i + _GROUPS_AHEAD
        for u in range(_GROUP_ROWS // _READ_ROWS):
            start_read(g, group_start(g) + u * _READ_ROWS)
        compute(i)
        wait_group(i + 1, group_start(i + 1), _GROUP_ROWS)

    start_group(n_groups, group_start(n_groups), _TAIL_ROWS)
    for g in range(n_early + 1, n_groups):
        wait_group(g, group_start(g), _GROUP_ROWS)

    pl.loop(0, _WRITES_AHEAD)(start_write)
    wait_group(n_groups, group_start(n_groups), _TAIL_ROWS)

    @pl.loop(n_early, n_blocks)
    def _(i):
        first = _WRITES_AHEAD + (i - n_early) * _WRITES_PER_STEP
        for u in range(_WRITES_PER_STEP):
            start_write(first + u)
        compute(i)

    pl.loop(n_paced, n_writes)(start_write)
    pltpu.make_async_copy(buf, o_hbm, aux_sem).wait()


@jax.jit
def pallas_standalone__dilated_atrous__vision_kernel(x: jax.Array, w: jax.Array):
    B, H, W, C = x.shape
    assert w.shape == (1, 1, C, C), "1x1 kernel with as many outputs as inputs"
    pixels = B * H * W
    length = pixels // _STREAMS
    assert length * _STREAMS == pixels
    assert length % _GROUP_ROWS == 0 and length % _WRITE_ROWS == 0

    out = pl.pallas_call(
        _conv1x1_kernel,
        in_specs=[
            pl.BlockSpec(memory_space=pl.ANY),
            pl.BlockSpec(memory_space=pl.ANY),
        ],
        out_specs=pl.BlockSpec(memory_space=pl.ANY),
        out_shape=jax.ShapeDtypeStruct((_STREAMS, length, C), x.dtype),
        scratch_shapes=[
            pltpu.VMEM((_STREAMS, length, C), x.dtype),
            pltpu.VMEM((C, C), w.dtype),
            pltpu.SemaphoreType.DMA((_GROUPS_AHEAD,)),
            pltpu.SemaphoreType.DMA,
        ],
        compiler_params=pltpu.CompilerParams(vmem_limit_bytes=118 * 1024 * 1024),
    )(x.reshape(_STREAMS, length, C), w.reshape(C, C))
    return out.reshape(B, H, W, C)
```
